```python
import os as _os
_os.environ.setdefault("JAX_PLATFORMS", "cpu")
import jax
import jax.numpy as jnp

def _softmax(x, axis=-1):
    return jax.nn.softmax(x, axis=axis)
def _gelu(x):
    return jax.nn.gelu(x, approximate=True)
def _silu(x):
    return jax.nn.silu(x)
def _sigmoid(x):
    return jax.nn.sigmoid(x)
def _layernorm(x, axis=-1, eps=1e-5):
    m = jnp.mean(x, axis=axis, keepdims=True)
    v = jnp.var(x, axis=axis, keepdims=True)
    return (x - m) / jnp.sqrt(v + eps)
def _scatter_add(tgt, idx, src, axis=0):
    return tgt.at[idx].add(src)
def _segment_sum(src, seg, n):
    return jax.ops.segment_sum(src, seg, n)
class _Rng:
    def __init__(self, key):
        self._k = key
    def _next(self):
        self._k, sub = jax.random.split(self._k)
        return sub
    def normal(self, shape):
        return jax.random.normal(self._next(), shape, dtype=jnp.bfloat16)
    def randint(self, lo, hi, shape):
        return jax.random.randint(self._next(), shape, lo, hi, dtype=jnp.int32)
    def uniform(self, shape, lo=0.0, hi=1.0):
        return jax.random.uniform(self._next(), shape, jnp.bfloat16, lo, hi)
    def permutation(self, n):
        return jax.random.permutation(self._next(), n)


kernel_name = 'standalone__mha_softmax__near_ridge'

def setup_inputs():
    _rng = _Rng(jax.random.key(int.from_bytes(__import__("os").urandom(4), "little")))
    _w = (lambda a: (lambda t: t.astype(jnp.bfloat16) if jnp.issubdtype(t.dtype, jnp.floating) else t)(jnp.asarray(a)))
    B, H, Sq, Sk, D = 8, 32, 304, 2048, 128
    return {
        "q": _w((lambda *s: _rng.normal(s) * 0.4)(B, H, Sq, D)),
        "k": _w((lambda *s: _rng.normal(s) * 0.4)(B, H, Sk, D)),
        "v": _w((lambda *s: _rng.normal(s) * 0.05)(B, H, Sk, D)),
    }

def reference(q, k, v):
    scale = q.shape[-1] ** -0.5
    scores = jnp.einsum("bhqd,bhkd->bhqk", q, k) * scale
    p = _softmax(scores, axis=-1)
    return jnp.einsum("bhqk,bhkd->bhqd", p, v)
```

```python
import functools

import jax
import jax.numpy as jnp
import jax.experimental.pallas as pl
import jax.experimental.pallas.tpu as pltpu


def _attn_kernel(q_ref, k_ref, v_ref, o_ref, *, scale, hb):
    for h in range(hb):
        q = q_ref[h]
        k = k_ref[h]
        v = v_ref[h]
        s = jax.lax.dot_general(
            q, k, (((1,), (1,)), ((), ())), preferred_element_type=jnp.float32
        ) * scale
        m = jnp.max(s, axis=1, keepdims=True)
        p = jnp.exp(s - m)
        l = jnp.sum(p, axis=1, keepdims=True)
        o = jnp.dot(p.astype(v.dtype), v, preferred_element_type=jnp.float32)
        o_ref[h] = (o / l).astype(o_ref.dtype)


@jax.jit
def pallas_standalone__mha_softmax__near_ridge_kernel(
    q: jax.Array,
    k: jax.Array,
    v: jax.Array,
):
    B, H, Sq, D = q.shape
    Sk = k.shape[2]
    scale = float(D) ** -0.5
    hb = 1
    grid = (B, H // hb)
    kern = functools.partial(_attn_kernel, scale=scale, hb=hb)
    return pl.pallas_call(
        kern,
        grid=grid,
        in_specs=[
            pl.BlockSpec((None, hb, Sq, D), lambda b, h: (b, h, 0, 0)),
            pl.BlockSpec((None, hb, Sk, D), lambda b, h: (b, h, 0, 0)),
            pl.BlockSpec((None, hb, Sk, D), lambda b, h: (b, h, 0, 0)),
        ],
        out_specs=pl.BlockSpec((None, hb, Sq, D), lambda b, h: (b, h, 0, 0)),
        out_shape=jax.ShapeDtypeStruct((B, H, Sq, D), q.dtype),
        compiler_params=pltpu.CompilerParams(
            dimension_semantics=("parallel", "parallel"),
            vmem_limit_bytes=64 * 1024 * 1024,
        ),
    )(q, k, v)
```

```python
import functools
import math

import jax
import jax.numpy as jnp
import jax.experimental.pallas as pl
import jax.experimental.pallas.tpu as pltpu

_LOG2E = math.log2(math.e)


def _qk(q, k):
    return jax.lax.dot_general(q, k, (((1,), (1,)), ((), ())),
                               preferred_element_type=jnp.float32)


def _two_pass_head(q, k, v):
    s = _qk(q, k)
    m = jnp.max(s, axis=1, keepdims=True)
    p = jnp.exp2(s - m)
    l = jnp.sum(p, axis=1, keepdims=True)
    o = jnp.dot(p.astype(v.dtype), v, preferred_element_type=jnp.float32)
    return o, l


def _online_head(q, k_ref, v_ref, nc):
    sk = k_ref.shape[0]
    ck = sk // nc
    m = l = acc = None
    for c in range(nc):
        kc = k_ref[c * ck:(c + 1) * ck]
        vc = v_ref[c * ck:(c + 1) * ck]
        s = _qk(q, kc)
        mc = jnp.max(s, axis=1, keepdims=True)
        m_new = mc if m is None else jnp.maximum(m, mc)
        p = jnp.exp2(s - m_new)
        lc = jnp.sum(p, axis=1, keepdims=True)
        oc = jnp.dot(p.astype(vc.dtype), vc, preferred_element_type=jnp.float32)
        if m is None:
            l, acc = lc, oc
        else:
            alpha = jnp.exp2(m - m_new)
            l = l * alpha + lc
            acc = acc * alpha + oc
        m = m_new
    return acc, l


def _attn_kernel(q_ref, k_ref, v_ref, o_ref, *, scale, hb, nc):
    c = scale * _LOG2E
    for h in range(hb):
        q = (q_ref[h].astype(jnp.float32) * c).astype(q_ref.dtype)
        if h == hb - 1 and nc > 1:
            o, l = _online_head(q, k_ref.at[h], v_ref.at[h], nc)
        else:
            o, l = _two_pass_head(q, k_ref[h], v_ref[h])
        o_ref[h] = (o * (1.0 / l)).astype(o_ref.dtype)


def _largest_divisor_at_most(n, cap):
    for d in range(min(cap, n), 0, -1):
        if n % d == 0:
            return d
    return 1


@jax.jit
def pallas_standalone__mha_softmax__near_ridge_kernel(
    q: jax.Array,
    k: jax.Array,
    v: jax.Array,
):
    B, H, Sq, D = q.shape
    Sk = k.shape[2]
    scale = float(D) ** -0.5
    hb = _largest_divisor_at_most(H, 8)
    nc = 4 if (Sk % 4 == 0 and (Sk // 4) % 16 == 0) else 1

    kernel = functools.partial(_attn_kernel, scale=scale, hb=hb, nc=nc)
    return pl.pallas_call(
        kernel,
        grid=(B, H // hb),
        in_specs=[
            pl.BlockSpec((None, hb, Sq, D), lambda b, h: (b, h, 0, 0)),
            pl.BlockSpec((None, hb, Sk, D), lambda b, h: (b, h, 0, 0)),
            pl.BlockSpec((None, hb, Sk, D), lambda b, h: (b, h, 0, 0)),
        ],
        out_specs=pl.BlockSpec((None, hb, Sq, D), lambda b, h: (b, h, 0, 0)),
        out_shape=jax.ShapeDtypeStruct((B, H, Sq, D), q.dtype),
        compiler_params=pltpu.CompilerParams(
            dimension_semantics=("parallel", "parallel"),
            vmem_limit_bytes=100 * 1024 * 1024,
        ),
    )(q, k, v)
```
